```python
import jax
import jax.numpy as jnp

def _softmax(x, axis=-1):
    return jax.nn.softmax(x, axis=axis)
def _gelu(x):
    return jax.nn.gelu(x, approximate=True)
def _silu(x):
    return jax.nn.silu(x)
def _sigmoid(x):
    return jax.nn.sigmoid(x)
def _layernorm(x, axis=-1, eps=1e-5):
    m = jnp.mean(x, axis=axis, keepdims=True)
    v = jnp.var(x, axis=axis, keepdims=True)
    return (x - m) / jnp.sqrt(v + eps)
def _scatter_add(tgt, idx, src, axis=0):
    return tgt.at[idx].add(src)
def _segment_sum(src, seg, n):
    return jax.ops.segment_sum(src, seg, n)
class _Rng:
    def __init__(self, key):
        self._k = key
    def _next(self):
        self._k, sub = jax.random.split(self._k)
        return sub
    def normal(self, shape):
        return jax.random.normal(self._next(), shape, dtype=jnp.bfloat16)
    def randint(self, lo, hi, shape):
        return jax.random.randint(self._next(), shape, lo, hi, dtype=jnp.int32)
    def uniform(self, shape, lo=0.0, hi=1.0):
        return jax.random.uniform(self._next(), shape, jnp.bfloat16, lo, hi)
    def permutation(self, n):
        return jax.random.permutation(self._next(), n)


kernel_name = 'interleave_layers__sliding_block__sliding_local_dilated__prompt'

def setup_inputs():
    _rng = _Rng(jax.random.key(int.from_bytes(__import__("os").urandom(4), "little")))
    _w = (lambda a: (lambda t: t.astype(jnp.bfloat16) if jnp.issubdtype(t.dtype, jnp.floating) else t)(jnp.asarray(a)))
    def _A_setup():
        B, S, D = 1, 2048, 1024
        return {
            "x": _w((lambda *s: _rng.normal(s) * 0.05)(B, S, D)),
            "wqkv": _w((lambda *s: _rng.normal(s) * 0.05)(D, 3 * D)),
            "wo": _w((lambda *s: _rng.normal(s) * 0.05)(D, D)),
        }
    _A_in = _A_setup()

    def _B_setup():
        B, S, D = 1, 2048, 1024
        return {
            "x": _w((lambda *s: _rng.normal(s) * 0.05)(B, S, D)),
            "wqkv": _w((lambda *s: _rng.normal(s) * 0.05)(D, 3 * D)),
            "wo": _w((lambda *s: _rng.normal(s) * 0.05)(D, D)),
        }
    _B_in = _B_setup()

    return {
        "A_x": _A_in["x"],
        "A_wqkv": _A_in["wqkv"],
        "A_wo": _A_in["wo"],
        "B_x": _B_in["x"],
        "B_wqkv": _B_in["wqkv"],
        "B_wo": _B_in["wo"],
    }

def reference(A_x, A_wqkv, A_wo, B_x, B_wqkv, B_wo):
    def _A_ref(x, wqkv, wo):
        B, S, D = x.shape
        H = 32; Dh = D // H; W = 256
        qkv = (lambda x, *d: x.transpose(*d))((x @ wqkv).reshape(B, S, 3, H, Dh), 2, 0, 3, 1, 4)
        q, k, v = qkv[0], qkv[1], qkv[2]
        scores = jnp.einsum("bhqd,bhkd->bhqk", q, k) * (Dh ** -0.5)
        idx = jnp.arange(S)
        mask = (idx[:, None] - idx[None, :] >= 0) & (idx[:, None] - idx[None, :] < W)
        scores = jnp.where(mask[None, None], scores, -1e9)
        p = _softmax(scores, axis=-1)
        o = jnp.einsum("bhqk,bhkd->bhqd", p, v)
        return (lambda x, *d: x.transpose(*d))(o, 0, 2, 1, 3).reshape(B, S, D) @ wo

    def _B_ref(x, wqkv, wo):
        B, S, D = x.shape
        H = 32; Dh = D // H
        W, dil = 8, 2
        qkv = (lambda x, *d: x.transpose(*d))((x @ wqkv).reshape(B, S, 3, H, Dh), 2, 0, 3, 1, 4)
        q, k, v = qkv[0], qkv[1], qkv[2]
        scale = Dh ** -0.5
        pos = jnp.arange(S)
        off = jnp.arange(W) * dil
        idx = pos[:, None] - off[None, :]
        mask = idx >= 0
        idx_c = jnp.where(mask, idx, 0).reshape(-1)
        kg = k[:, :, idx_c, :].reshape(B, H, S, W, Dh)
        vg = v[:, :, idx_c, :].reshape(B, H, S, W, Dh)
        logits = jnp.einsum("bhsd,bhswd->bhsw", q, kg) * scale
        logits = jnp.where(mask[None, None, :, :], logits, -1e9)
        attn = _softmax(logits, axis=-1)
        o = jnp.einsum("bhsw,bhswd->bhsd", attn, vg)
        return (lambda x, *d: x.transpose(*d))(o, 0, 2, 1, 3).reshape(B, S, D) @ wo

    x = A_x
    x = x + _A_ref(_layernorm(x, axis=-1), A_wqkv, A_wo)
    x = x + _B_ref(_layernorm(x, axis=-1), B_wqkv, B_wo)
    x = x + _A_ref(_layernorm(x, axis=-1), A_wqkv, A_wo)
    x = x + _B_ref(_layernorm(x, axis=-1), B_wqkv, B_wo)
    return x
```

```python
import math

import jax
import jax.numpy as jnp
import jax.experimental.pallas as pl
import jax.experimental.pallas.tpu as pltpu

S = 2048
D = 1024
H = 32
DH = 32
WA = 256
PAD = 256
QB = 128
MB = 512
NEG = -1e9
LOG2E = 1.4426950408889634
QSCALE = (DH ** -0.5) * LOG2E

_NT = (((1,), (1,)), ((), ()))
_TN = (((0,), (0,)), ((), ()))


def _kernel(x_ref, awqkv_ref, awo_ref, bwqkv_ref, bwo_ref, out_ref,
            xr_ref, q_ref, k_ref, vt_ref):
    f32, bf16 = jnp.float32, jnp.bfloat16

    k_ref[0:PAD, :] = jnp.zeros((PAD, D), bf16)
    vt_ref[:, 0:PAD] = jnp.zeros((D, PAD), bf16)

    def load_x(i, c):
        r = pl.ds(pl.multiple_of(i * MB, MB), MB)
        xr_ref[r, :] = x_ref[r, :].astype(f32)
        return c
    jax.lax.fori_loop(0, S // MB, load_x, 0)

    def qkv_phase(w_ref):
        def body(i, c):
            r0 = pl.multiple_of(i * MB, MB)
            x = xr_ref[pl.ds(r0, MB), :]
            m = jnp.mean(x, axis=-1, keepdims=True)
            xc = x - m
            v = jnp.mean(xc * xc, axis=-1, keepdims=True)
            xn = (xc * jax.lax.rsqrt(v + 1e-5)).astype(bf16)
            q = jnp.dot(xn, w_ref[:, 0:D], preferred_element_type=f32)
            q_ref[pl.ds(r0, MB), :] = (q * QSCALE).astype(bf16)
            k = jnp.dot(xn, w_ref[:, D:2 * D], preferred_element_type=f32)
            k_ref[pl.ds(PAD + r0, MB), :] = k.astype(bf16)
            vv = jnp.dot(xn, w_ref[:, 2 * D:3 * D], preferred_element_type=f32)
            vt_ref[:, pl.ds(PAD + r0, MB)] = vv.astype(bf16).T
            return c
        jax.lax.fori_loop(0, S // MB, body, 0)

    lane = jax.lax.broadcasted_iota(jnp.int32, (QB, QB), 1)
    row = jax.lax.broadcasted_iota(jnp.int32, (QB, QB), 0)

    def softmax_cols(tiles):
        mx = None
        for t in tiles:
            tm = jnp.max(t, axis=0, keepdims=True)
            mx = tm if mx is None else jnp.maximum(mx, tm)
        ps = [jnp.exp2(t - mx) for t in tiles]
        sm = None
        for p in ps:
            t = jnp.sum(p, axis=0, keepdims=True)
            sm = t if sm is None else sm + t
        return ps, 1.0 / sm

    def attn_phase(wo_ref, is_a, last):
        def body(i, c):
            r0 = pl.multiple_of(i * QB, QB)
            if is_a:
                nk = QB + WA
                k0 = pl.multiple_of(r0 + PAD - WA, QB)
                tri = row <= lane
                old_ok = i >= 2
                mid_ok = i >= 1
            else:
                nk = 2 * QB
                k0 = pl.multiple_of(r0 + PAD - QB, QB)
                c2 = jax.lax.broadcasted_iota(jnp.int32, (QB + 16, QB), 0)
                l2 = jax.lax.broadcasted_iota(jnp.int32, (QB + 16, QB), 1)
                dist = l2 + 16 - c2
                bmask = ((dist >= 0) & (dist < 16) & ((dist & 1) == 0)
                         & (c2 + r0 >= 16))
            ots = []
            for g in range(H // 4):
                cols = slice(g * 128, (g + 1) * 128)
                qg = q_ref[pl.ds(r0, QB), cols]
                if is_a:
                    kg = k_ref[pl.ds(k0, nk), cols]
                else:
                    kg = k_ref[pl.ds(pl.multiple_of(r0 + PAD - 16, 16), QB + 16), cols]
                for hh in range(4):
                    h = g * 4 + hh
                    hm = (lane >= hh * DH) & (lane < (hh + 1) * DH)
                    qh = jnp.where(hm, qg, jnp.zeros_like(qg))
                    st = jax.lax.dot_general(kg, qh, _NT, preferred_element_type=f32)
                    vth = vt_ref[h * DH:(h + 1) * DH, pl.ds(k0, nk)]
                    if is_a:
                        s_old = jnp.where(old_ok, st[0:QB], NEG)
                        s_mid = jnp.where(mid_ok, st[QB:2 * QB], NEG)
                        s_mrg = jnp.where(tri, st[2 * QB:3 * QB], s_old)
                        (p_mrg, p_mid), inv = softmax_cols([s_mrg, s_mid])
                        zero = jnp.zeros_like(p_mrg)
                        p = jnp.concatenate([jnp.where(tri, zero, p_mrg), p_mid,
                                             jnp.where(tri, p_mrg, zero)], axis=0)
                    else:
                        (pb,), inv = softmax_cols([jnp.where(bmask, st, NEG)])
                        p = jnp.concatenate([jnp.zeros((QB - 16, QB), f32), pb], axis=0)
                    ot = jnp.dot(vth, p.astype(bf16), preferred_element_type=f32)
                    ots.append((ot * inv).astype(bf16))
            ot_all = jnp.concatenate(ots, axis=0)
            y = jax.lax.dot_general(ot_all, wo_ref[...], _TN, preferred_element_type=f32)
            xnew = xr_ref[pl.ds(r0, QB), :] + y
            xr_ref[pl.ds(r0, QB), :] = xnew
            if last:
                out_ref[pl.ds(r0, QB), :] = xnew.astype(bf16)
            return c
        jax.lax.fori_loop(0, S // QB, body, 0)

    qkv_phase(awqkv_ref)
    attn_phase(awo_ref, True, False)
    qkv_phase(bwqkv_ref)
    attn_phase(bwo_ref, False, False)
    qkv_phase(awqkv_ref)
    attn_phase(awo_ref, True, False)
    qkv_phase(bwqkv_ref)
    attn_phase(bwo_ref, False, True)


@jax.jit
def pallas_interleave_layers__sliding_block__sliding_local_dilated__prompt_kernel(
    A_x: jax.Array,
    A_wqkv: jax.Array,
    A_wo: jax.Array,
    B_x: jax.Array,
    B_wqkv: jax.Array,
    B_wo: jax.Array,
):
    del B_x
    x = A_x.reshape(S, D)
    out = pl.pallas_call(
        _kernel,
        out_shape=jax.ShapeDtypeStruct((S, D), jnp.bfloat16),
        scratch_shapes=[
            pltpu.VMEM((S, D), jnp.float32),
            pltpu.VMEM((S, D), jnp.bfloat16),
            pltpu.VMEM((PAD + S, D), jnp.bfloat16),
            pltpu.VMEM((D, PAD + S), jnp.bfloat16),
        ],
        compiler_params=pltpu.CompilerParams(vmem_limit_bytes=100 * 1024 * 1024),
    )(x, A_wqkv, A_wo, B_wqkv, B_wo)
    return out.reshape(1, S, D)
```

```python
import math

import jax
import jax.numpy as jnp
import jax.experimental.pallas as pl
import jax.experimental.pallas.tpu as pltpu

S = 2048
D = 1024
H = 32
DH = 32
WA = 256
PAD = 256
QB = 128
MB = 512
NEG = -1e9
LOG2E = 1.4426950408889634
QSCALE = (DH ** -0.5) * LOG2E

_NT = (((1,), (1,)), ((), ()))
_TN = (((0,), (0,)), ((), ()))


def _kernel(x_ref, awqkv_ref, awo_ref, bwqkv_ref, bwo_ref, out_ref,
            xr_ref, xn_ref, q_ref, k_ref, vt_ref, st_ref, o_ref):
    f32, bf16 = jnp.float32, jnp.bfloat16

    k_ref[0:PAD, :] = jnp.zeros((PAD, D), bf16)
    vt_ref[:, 0:PAD] = jnp.zeros((D, PAD), bf16)

    def layernorm(x):
        m = jnp.mean(x, axis=-1, keepdims=True)
        xc = x - m
        v = jnp.mean(xc * xc, axis=-1, keepdims=True)
        return (xc * jax.lax.rsqrt(v + 1e-5)).astype(bf16)

    def load_x(i, c):
        r = pl.ds(pl.multiple_of(i * QB, QB), QB)
        x = x_ref[r, :].astype(f32)
        xr_ref[r, :] = x
        xn_ref[r, :] = layernorm(x)
        return c
    jax.lax.fori_loop(0, S // QB, load_x, 0)

    def qkv_phase(w_ref):
        def body(i, c):
            r0 = pl.multiple_of(i * MB, MB)
            xn = xn_ref[pl.ds(r0, MB), :]
            vv = jnp.dot(xn, w_ref[:, 2 * D:3 * D], preferred_element_type=f32)
            vt_ref[:, pl.ds(PAD + r0, MB)] = vv.astype(bf16).T
            q = jnp.dot(xn, w_ref[:, 0:D], preferred_element_type=f32)
            q_ref[pl.ds(r0, MB), :] = (q * QSCALE).astype(bf16)
            k = jnp.dot(xn, w_ref[:, D:2 * D], preferred_element_type=f32)
            k_ref[pl.ds(PAD + r0, MB), :] = k.astype(bf16)
            return c
        jax.lax.fori_loop(0, S // MB, body, 0)

    lane = jax.lax.broadcasted_iota(jnp.int32, (QB, QB), 1)
    row = jax.lax.broadcasted_iota(jnp.int32, (QB, QB), 0)

    def softmax_cols(tiles):
        mx = None
        for t in tiles:
            tm = jnp.max(t, axis=0, keepdims=True)
            mx = tm if mx is None else jnp.maximum(mx, tm)
        ps = [jnp.exp2(t - mx) for t in tiles]
        sm = None
        for p in ps:
            t = jnp.sum(p, axis=0, keepdims=True)
            sm = t if sm is None else sm + t
        return ps, 1.0 / sm

    NG = H // 4

    def attn_phase(wo_ref, is_a, last):
        nk = QB + WA if is_a else QB + 16
        nv = QB + WA if is_a else 2 * QB

        o_ref[1] = jnp.zeros((QB, D), bf16)

        def krows(r0):
            if is_a:
                return pl.ds(pl.multiple_of(r0 + PAD - WA, QB), nk)
            return pl.ds(pl.multiple_of(r0 + PAD - 16, 16), nk)

        def qk(r0, g):
            cols = slice(g * 128, (g + 1) * 128)
            qg = q_ref[pl.ds(r0, QB), cols]
            kg = k_ref[krows(r0), cols]
            zq = jnp.zeros_like(qg)
            qm = jnp.concatenate(
                [jnp.where((lane >= hh * DH) & (lane < (hh + 1) * DH), qg, zq)
                 for hh in range(4)], axis=0)
            st_ref[g % 2, 0:nk, :] = jax.lax.dot_general(
                kg, qm, _NT, preferred_element_type=f32)

        def finish_rows(r):
            x = xr_ref[r, :]
            if last:
                out_ref[r, :] = x.astype(bf16)
            else:
                xn_ref[r, :] = layernorm(x)

        def body(i, c):
            r0 = pl.multiple_of(i * QB, QB)
            rn = pl.multiple_of(jnp.minimum(i + 1, S // QB - 1) * QB, QB)
            rp = pl.ds(pl.multiple_of(jnp.maximum(i - 1, 0) * QB, QB), QB)
            if is_a:
                v0 = pl.multiple_of(r0 + PAD - WA, QB)
                tri = row <= lane
                old_ok = i >= 2
                mid_ok = i >= 1
            else:
                v0 = pl.multiple_of(r0 + PAD - QB, QB)
                c2 = jax.lax.broadcasted_iota(jnp.int32, (QB + 16, QB), 0)
                l2 = jax.lax.broadcasted_iota(jnp.int32, (QB + 16, QB), 1)
                dist = l2 + 16 - c2
                bmask = ((dist >= 0) & (dist < 16) & ((dist & 1) == 0)
                         & (c2 + r0 >= 16))

            def sm_pv(g, slot):
                ots = []
                for hh in range(4):
                    h = g * 4 + hh
                    hc = slice(hh * 128, (hh + 1) * 128)
                    vth = vt_ref[h * DH:(h + 1) * DH, pl.ds(v0, nv)]
                    if is_a:
                        s_old = jnp.where(old_ok, st_ref[g % 2, 0:QB, hc], NEG)
                        s_mid = jnp.where(mid_ok, st_ref[g % 2, QB:2 * QB, hc], NEG)
                        s_mrg = jnp.where(tri, st_ref[g % 2, 2 * QB:3 * QB, hc], s_old)
                        (p_mrg, p_mid), inv = softmax_cols([s_mrg, s_mid])
                        zero = jnp.zeros_like(p_mrg)
                        p = jnp.concatenate([jnp.where(tri, zero, p_mrg), p_mid,
                                             jnp.where(tri, p_mrg, zero)], axis=0)
                    else:
                        sb = jnp.where(bmask, st_ref[g % 2, 0:nk, hc], NEG)
                        (pb,), inv = softmax_cols([sb])
                        p = jnp.concatenate([jnp.zeros((QB - 16, QB), f32), pb], axis=0)
                    ot = jnp.dot(vth, p.astype(bf16), preferred_element_type=f32)
                    ots.append((ot * inv).astype(bf16))
                ot_g = jnp.concatenate(ots, axis=0)
                o_ref[slot, :, g * 128:(g + 1) * 128] = ot_g.T

            slot = i % 2
            for g in range(NG):
                if g + 1 < NG:
                    qk(r0, g + 1)
                cols = slice(g * 128, (g + 1) * 128)
                y = jnp.dot(o_ref[1 - slot], wo_ref[:, cols], preferred_element_type=f32)
                xr_ref[rp, cols] = xr_ref[rp, cols] + y
                if g + 1 == NG:
                    finish_rows(rp)
                sm_pv(g, slot)
            qk(rn, 0)
            return c
        qk(0, 0)
        jax.lax.fori_loop(0, S // QB, body, 0)
        r = pl.ds(S - QB, QB)
        xr_ref[r, :] = xr_ref[r, :] + jnp.dot(o_ref[(S // QB - 1) % 2], wo_ref[...],
                                              preferred_element_type=f32)
        finish_rows(r)

    qkv_phase(awqkv_ref)
    attn_phase(awo_ref, True, False)
    qkv_phase(bwqkv_ref)
    attn_phase(bwo_ref, False, False)
    qkv_phase(awqkv_ref)
    attn_phase(awo_ref, True, False)
    qkv_phase(bwqkv_ref)
    attn_phase(bwo_ref, False, True)


@jax.jit
def pallas_interleave_layers__sliding_block__sliding_local_dilated__prompt_kernel(
    A_x: jax.Array,
    A_wqkv: jax.Array,
    A_wo: jax.Array,
    B_x: jax.Array,
    B_wqkv: jax.Array,
    B_wo: jax.Array,
):
    del B_x
    x = A_x.reshape(S, D)
    out = pl.pallas_call(
        _kernel,
        out_shape=jax.ShapeDtypeStruct((S, D), jnp.bfloat16),
        scratch_shapes=[
            pltpu.VMEM((S, D), jnp.float32),
            pltpu.VMEM((S, D), jnp.bfloat16),
            pltpu.VMEM((S, D), jnp.bfloat16),
            pltpu.VMEM((PAD + S, D), jnp.bfloat16),
            pltpu.VMEM((D, PAD + S), jnp.bfloat16),
            pltpu.VMEM((2, QB + WA, 4 * QB), jnp.float32),
            pltpu.VMEM((2, QB, D), jnp.bfloat16),
        ],
        compiler_params=pltpu.CompilerParams(vmem_limit_bytes=100 * 1024 * 1024),
    )(x, A_wqkv, A_wo, B_wqkv, B_wo)
    return out.reshape(1, S, D)
```

```python
import math

import jax
import jax.numpy as jnp
import jax.experimental.pallas as pl
import jax.experimental.pallas.tpu as pltpu

S = 2048
D = 1024
H = 32
DH = 32
WA = 256
PAD = 256
QB = 128
MB = 512
NEG = -1e9
LOG2E = 1.4426950408889634
QSCALE = (DH ** -0.5) * LOG2E

_NT = (((1,), (1,)), ((), ()))
_TN = (((0,), (0,)), ((), ()))


def _kernel(x_hbm, awqkv_hbm, awo_hbm, bwqkv_hbm, bwo_hbm, out_hbm,
            awqkv_ref, awo_ref, bwqkv_ref, bwo_ref, sems,
            xr_ref, xn_ref, q_ref, k_ref, vt_ref, st0_ref, st1_ref, mx0_ref, mx1_ref, o_ref):
    st_refs, mx_refs = (st0_ref, st1_ref), (mx0_ref, mx1_ref)
    f32, bf16 = jnp.float32, jnp.bfloat16

    nxc = S // MB
    x_cp = [pltpu.make_async_copy(x_hbm.at[c * MB:(c + 1) * MB], xn_ref.at[c * MB:(c + 1) * MB],
                                  sems.at[c]) for c in range(nxc)]
    w_cp = [pltpu.make_async_copy(awqkv_hbm.at[:, t * D:(t + 1) * D],
                                  awqkv_ref.at[:, t * D:(t + 1) * D], sems.at[nxc + t])
            for t in range(3)]
    awo_cp = pltpu.make_async_copy(awo_hbm, awo_ref, sems.at[nxc + 3])
    bw_cp = pltpu.make_async_copy(bwqkv_hbm, bwqkv_ref, sems.at[nxc + 4])
    bwo_cp = pltpu.make_async_copy(bwo_hbm, bwo_ref, sems.at[nxc + 5])
    out_sem = sems.at[nxc + 6]

    def out_cp(blk):
        r = pl.ds(pl.multiple_of(blk * QB, QB), QB)
        return pltpu.make_async_copy(xn_ref.at[r], out_hbm.at[r], out_sem)

    x_cp[0].start()
    w_cp[2].start()
    for c in range(1, nxc):
        x_cp[c].start()
    w_cp[0].start()
    w_cp[1].start()

    k_ref[0:PAD, :] = jnp.zeros((PAD, D), bf16)
    vt_ref[:, 0:PAD] = jnp.zeros((D, PAD), bf16)

    def layernorm(x):
        m = jnp.mean(x, axis=-1, keepdims=True)
        xc = x - m
        v = jnp.mean(xc * xc, axis=-1, keepdims=True)
        return (xc * jax.lax.rsqrt(v + 1e-5)).astype(bf16)

    def load_x(i, c):
        r = pl.ds(pl.multiple_of(i * QB, QB), QB)
        x = xn_ref[r, :].astype(f32)
        xr_ref[r, :] = x
        xn_ref[r, :] = layernorm(x)
        return c
    for c in range(nxc):
        x_cp[c].wait()
        jax.lax.fori_loop(c * (MB // QB), (c + 1) * (MB // QB), load_x, 0)
    awo_cp.start()
    bw_cp.start()
    bwo_cp.start()

    def qkv_phase(w_ref, first=False):
        def body(i, c):
            r0 = pl.multiple_of(i * MB, MB)
            xn = xn_ref[pl.ds(r0, MB), :]
            vv = jnp.dot(xn, w_ref[:, 2 * D:3 * D], preferred_element_type=f32)
            vt_ref[:, pl.ds(PAD + r0, MB)] = vv.astype(bf16).T
            if first:
                pl.when(i == 0)(lambda: (w_cp[0].wait(), w_cp[1].wait()) and None)
            q = jnp.dot(xn, w_ref[:, 0:D], preferred_element_type=f32)
            q_ref[pl.ds(r0, MB), :] = (q * QSCALE).astype(bf16)
            k = jnp.dot(xn, w_ref[:, D:2 * D], preferred_element_type=f32)
            k_ref[pl.ds(PAD + r0, MB), :] = k.astype(bf16)
            return c
        jax.lax.fori_loop(0, S // MB, body, 0)

    lane = jax.lax.broadcasted_iota(jnp.int32, (QB, QB), 1)
    row = jax.lax.broadcasted_iota(jnp.int32, (QB, QB), 0)

    NG = H // 4
    lane_h = jax.lax.broadcasted_iota(jnp.int32, (QB // 2, QB), 1)
    row_h = jax.lax.broadcasted_iota(jnp.int32, (QB // 2, QB), 0)

    def attn_phase(wo_ref, is_a, last):
        nk = QB + WA if is_a else QB + 16
        nv = QB + WA if is_a else 2 * QB

        o_ref[1] = jnp.zeros((QB, D), bf16)

        def qk(i, g):
            r0 = pl.multiple_of(i * QB, QB)
            st_ref, mx_ref = st_refs[g % 2], mx_refs[g % 2]
            z = i >> 11
            cols = slice(g * 128, (g + 1) * 128)
            qg = q_ref[pl.ds(r0, QB), cols]
            qu = pltpu.bitcast(qg, jnp.uint32)
            qm = jnp.concatenate(
                [pltpu.bitcast(jnp.where((lane_h >> 5) == hh, qu, jnp.uint32(0)), bf16)
                 for hh in range(4)], axis=0)
            if is_a:
                k_old = k_ref[pl.ds(r0 + PAD - WA, QB), cols]
                k_mid = k_ref[pl.ds(r0 + PAD - QB, QB), cols]
                k_dia = k_ref[pl.ds(r0 + PAD, QB), cols]
                parts = []
                for t in range(QB // 16):
                    parts += [k_old[16 * t:16 * t + 16], k_dia[16 * t:16 * t + 16]]
                kg = jnp.concatenate(parts + [k_mid], axis=0)
            else:
                kg = k_ref[pl.ds(pl.multiple_of(r0 + PAD - 16, 16), nk), cols]
                c2 = jax.lax.broadcasted_iota(jnp.int32, (QB + 16, QB), 0)
                l2 = jax.lax.broadcasted_iota(jnp.int32, (QB + 16, QB), 1)
                dist = l2 + 16 - c2
                bmask = ((dist >= 0) & (dist < 16) & ((dist & 1) == 0)
                         & (c2 + r0 >= 16))
            st = jax.lax.dot_general(kg, qm, _NT, preferred_element_type=f32)
            mxs = [None] * 4

            def keep(hh, rows, sm):
                st_ref[z, rows, hh * 128:(hh + 1) * 128] = sm
                m8 = jnp.maximum(sm[0:8], sm[8:16])
                mxs[hh] = m8 if mxs[hh] is None else jnp.maximum(mxs[hh], m8)

            if is_a:
                for t in range(QB // 16):
                    tri = (row <= lane)[16 * t:16 * t + 16]
                    for hh in range(4):
                        hc = slice(hh * 128, (hh + 1) * 128)
                        s_old = jnp.where(i >= 2, st[32 * t:32 * t + 16, hc], NEG)
                        keep(hh, slice(16 * t, 16 * t + 16),
                             jnp.where(tri, st[32 * t + 16:32 * t + 32, hc], s_old))
                for t in range(QB // 16):
                    for hh in range(4):
                        hc = slice(hh * 128, (hh + 1) * 128)
                        keep(hh, slice(QB + 16 * t, QB + 16 * t + 16),
                             jnp.where(i >= 1, st[2 * QB + 16 * t:2 * QB + 16 * t + 16, hc], NEG))
            else:
                for t in range(nk // 16):
                    for hh in range(4):
                        hc = slice(hh * 128, (hh + 1) * 128)
                        keep(hh, slice(16 * t, 16 * t + 16),
                             jnp.where(bmask[16 * t:16 * t + 16], st[16 * t:16 * t + 16, hc], NEG))
            for hh in range(4):
                mx_ref[z, :, hh * 128:(hh + 1) * 128] = jnp.broadcast_to(
                    jnp.max(mxs[hh], axis=0, keepdims=True), (8, QB))

        def finish_rows(r):
            x = xr_ref[r, :]
            xn_ref[r, :] = x.astype(bf16) if last else layernorm(x)

        def body(i, c):
            if last:
                pl.when(i >= 2)(lambda: out_cp(i - 2).start())
            r0 = pl.multiple_of(i * QB, QB)
            rp = pl.ds(pl.multiple_of(jnp.maximum(i - 1, 0) * QB, QB), QB)
            v0 = pl.multiple_of(r0 + PAD - (WA if is_a else QB), QB)

            def sm_pv(g, slot):
                st_ref, mx_ref = st_refs[g % 2], mx_refs[g % 2]
                z = i >> 12
                ots = []
                for hh in range(4):
                    h = g * 4 + hh
                    hc = slice(hh * 128, (hh + 1) * 128)
                    vth = vt_ref[h * DH:(h + 1) * DH, pl.ds(v0, nv)]
                    mx = mx_ref[z, 0:1, hc]
                    ns = 2 * QB if is_a else nk
                    pe = jnp.exp2(st_ref[z, 0:ns, hc] - mx)
                    inv = 1.0 / jnp.sum(pe, axis=0, keepdims=True)
                    if is_a:
                        tri = row <= lane
                        p = jnp.concatenate([jnp.where(tri, 0.0, pe[0:QB]), pe[QB:],
                                             jnp.where(tri, pe[0:QB], 0.0)], axis=0)
                    else:
                        p = jnp.concatenate([jnp.zeros((QB - 16, QB), f32), pe], axis=0)
                    ot = jnp.dot(vth, p.astype(bf16), preferred_element_type=f32)
                    ots.append(ot * inv)
                ot_g = jnp.concatenate(ots, axis=0)
                o_ref[slot, :, g * 128:(g + 1) * 128] = ot_g.T.astype(bf16)

            slot = i % 2
            for g in range(NG):
                if g + 1 < NG:
                    qk(i, g + 1)
                cols = slice(g * 128, (g + 1) * 128)
                y = jnp.dot(o_ref[1 - slot], wo_ref[:, cols], preferred_element_type=f32)
                xr_ref[rp, cols] = xr_ref[rp, cols] + y
                if g + 1 == NG:
                    finish_rows(rp)
                sm_pv(g, slot)
            qk(jnp.minimum(i + 1, S // QB - 1), 0)
            return c
        qk(pl.program_id(0), 0)
        jax.lax.fori_loop(0, S // QB, body, 0)
        if last:
            out_cp(S // QB - 2).start()
        r = pl.ds(S - QB, QB)
        xr_ref[r, :] = xr_ref[r, :] + jnp.dot(o_ref[(S // QB - 1) % 2], wo_ref[...],
                                              preferred_element_type=f32)
        finish_rows(r)
        if last:
            out_cp(S // QB - 1).start()
            pltpu.make_async_copy(xn_ref, out_hbm, out_sem).wait()

    w_cp[2].wait()
    qkv_phase(awqkv_ref, first=True)
    awo_cp.wait()
    attn_phase(awo_ref, True, False)
    bw_cp.wait()
    bwo_cp.wait()
    qkv_phase(bwqkv_ref)
    attn_phase(bwo_ref, False, False)
    qkv_phase(awqkv_ref)
    attn_phase(awo_ref, True, False)
    qkv_phase(bwqkv_ref)
    attn_phase(bwo_ref, False, True)


@jax.jit
def pallas_interleave_layers__sliding_block__sliding_local_dilated__prompt_kernel(
    A_x: jax.Array,
    A_wqkv: jax.Array,
    A_wo: jax.Array,
    B_x: jax.Array,
    B_wqkv: jax.Array,
    B_wo: jax.Array,
):
    del B_x
    x = A_x.reshape(S, D)
    out = pl.pallas_call(
        _kernel,
        grid=(1,),
        in_specs=[pl.BlockSpec(memory_space=pl.ANY)] * 5,
        out_specs=pl.BlockSpec(memory_space=pl.ANY),
        out_shape=jax.ShapeDtypeStruct((S, D), jnp.bfloat16),
        scratch_shapes=[
            pltpu.VMEM((D, 3 * D), jnp.bfloat16),
            pltpu.VMEM((D, D), jnp.bfloat16),
            pltpu.VMEM((D, 3 * D), jnp.bfloat16),
            pltpu.VMEM((D, D), jnp.bfloat16),
            pltpu.SemaphoreType.DMA((S // MB + 7,)),
            pltpu.VMEM((S, D), jnp.float32),
            pltpu.VMEM((S, D), jnp.bfloat16),
            pltpu.VMEM((S, D), jnp.bfloat16),
            pltpu.VMEM((PAD + S, D), jnp.bfloat16),
            pltpu.VMEM((D, PAD + S), jnp.bfloat16),
            pltpu.VMEM((2, 2 * QB, 4 * QB), jnp.float32),
            pltpu.VMEM((2, 2 * QB, 4 * QB), jnp.float32),
            pltpu.VMEM((2, 8, 4 * QB), jnp.float32),
            pltpu.VMEM((2, 8, 4 * QB), jnp.float32),
            pltpu.VMEM((2, QB, D), jnp.bfloat16),
        ],
        compiler_params=pltpu.CompilerParams(vmem_limit_bytes=100 * 1024 * 1024),
    )(x, A_wqkv, A_wo, B_wqkv, B_wo)
    return out.reshape(1, S, D)
```

```python
import math

import jax
import jax.numpy as jnp
import jax.experimental.pallas as pl
import jax.experimental.pallas.tpu as pltpu

S = 2048
D = 1024
H = 32
DH = 32
WA = 256
PAD = 256
QB = 128
HQ = 64
MB = 512
NEG = -1e9
LOG2E = 1.4426950408889634
QSCALE = (DH ** -0.5) * LOG2E

_NT = (((1,), (1,)), ((), ()))
_TN = (((0,), (0,)), ((), ()))


def _kernel(x_hbm, awqkv_hbm, awo_hbm, bwqkv_hbm, bwo_hbm, out_hbm,
            awqkv_ref, awo_ref, bwqkv_ref, bwo_ref, sems,
            xr_ref, xn_ref, q_ref, k_ref, vt_ref, st0_ref, st1_ref, mx0_ref, mx1_ref, o_ref):
    st_refs, mx_refs = (st0_ref, st1_ref), (mx0_ref, mx1_ref)
    f32, bf16 = jnp.float32, jnp.bfloat16

    nxc = S // MB
    x_cp = [pltpu.make_async_copy(x_hbm.at[c * MB:(c + 1) * MB], xn_ref.at[c * MB:(c + 1) * MB],
                                  sems.at[c]) for c in range(nxc)]
    w_cp = [pltpu.make_async_copy(awqkv_hbm.at[:, t * D:(t + 1) * D],
                                  awqkv_ref.at[:, t * D:(t + 1) * D], sems.at[nxc + t])
            for t in range(3)]
    awo_cp = pltpu.make_async_copy(awo_hbm, awo_ref, sems.at[nxc + 3])
    bw_cp = pltpu.make_async_copy(bwqkv_hbm, bwqkv_ref, sems.at[nxc + 4])
    bwo_cp = pltpu.make_async_copy(bwo_hbm, bwo_ref, sems.at[nxc + 5])
    out_sem = sems.at[nxc + 6]

    def out_cp(blk):
        r = pl.ds(pl.multiple_of(blk * QB, QB), QB)
        return pltpu.make_async_copy(xn_ref.at[r], out_hbm.at[r], out_sem)

    x_cp[0].start()
    w_cp[2].start()
    for c in range(1, nxc):
        x_cp[c].start()
    w_cp[0].start()
    w_cp[1].start()

    k_ref[0:PAD, :] = jnp.zeros((PAD, D), bf16)
    vt_ref[:, 0:PAD] = jnp.zeros((D, PAD), bf16)

    def layernorm(x):
        m = jnp.mean(x, axis=-1, keepdims=True)
        xc = x - m
        v = jnp.mean(xc * xc, axis=-1, keepdims=True)
        return (xc * jax.lax.rsqrt(v + 1e-5)).astype(bf16)

    def load_x(i, c):
        r = pl.ds(pl.multiple_of(i * QB, QB), QB)
        x = xn_ref[r, :].astype(f32)
        xr_ref[r, :] = x
        xn_ref[r, :] = layernorm(x)
        return c
    for c in range(nxc):
        x_cp[c].wait()
        jax.lax.fori_loop(c * (MB // QB), (c + 1) * (MB // QB), load_x, 0)
    awo_cp.start()
    bw_cp.start()
    bwo_cp.start()

    def qkv_phase(w_ref, first=False):
        def body(i, c):
            r0 = pl.multiple_of(i * MB, MB)
            xn = xn_ref[pl.ds(r0, MB), :]
            vv = jnp.dot(xn, w_ref[:, 2 * D:3 * D], preferred_element_type=f32)
            vt_ref[:, pl.ds(PAD + r0, MB)] = vv.astype(bf16).T
            if first:
                pl.when(i == 0)(lambda: (w_cp[0].wait(), w_cp[1].wait()) and None)
            q = jnp.dot(xn, w_ref[:, 0:D], preferred_element_type=f32)
            q_ref[pl.ds(r0, MB), :] = (q * QSCALE).astype(bf16)
            k = jnp.dot(xn, w_ref[:, D:2 * D], preferred_element_type=f32)
            k_ref[pl.ds(PAD + r0, MB), :] = k.astype(bf16)
            return c
        jax.lax.fori_loop(0, S // MB, body, 0)

    lane = jax.lax.broadcasted_iota(jnp.int32, (QB, QB), 1)
    row = jax.lax.broadcasted_iota(jnp.int32, (QB, QB), 0)

    NG = H // 4
    lane_q = jax.lax.broadcasted_iota(jnp.int32, (HQ // 2, QB), 1)
    lane_q2 = jax.lax.broadcasted_iota(jnp.int32, (HQ, QB), 1)
    row_q = jax.lax.broadcasted_iota(jnp.int32, (HQ, QB), 0)
    ql16 = jax.lax.broadcasted_iota(jnp.int32, (16, QB), 1) & (HQ - 1)
    row16 = jax.lax.broadcasted_iota(jnp.int32, (16, QB), 0)

    def attn_phase(wo_ref, is_a, last):
        nk = HQ + WA if is_a else HQ + 16
        ns = WA if is_a else nk
        nv = QB + WA if is_a else 2 * QB

        def qk(i, g):
            r0 = pl.multiple_of(i * QB, QB)
            st_ref, mx_ref = st_refs[g % 2], mx_refs[g % 2]
            z = i >> 11
            cols = slice(g * 128, (g + 1) * 128)
            sts = []
            for j in range(2):
                qu = pltpu.bitcast(q_ref[pl.ds(r0 + HQ * j, HQ), cols], jnp.uint32)
                qm = jnp.concatenate(
                    [pltpu.bitcast(jnp.where((lane_q >> 5) == (hh ^ j), qu, jnp.uint32(0)), bf16)
                     for hh in range(4)], axis=0)
                kb = r0 + PAD + HQ * j
                if is_a:
                    k_old = k_ref[pl.ds(kb - WA, HQ), cols]
                    k_dia = k_ref[pl.ds(kb, HQ), cols]
                    parts = []
                    for t in range(HQ // 16):
                        parts += [k_old[16 * t:16 * t + 16], k_dia[16 * t:16 * t + 16]]
                    parts.append(k_ref[pl.ds(kb - WA + HQ, WA - HQ), cols])
                    kg = jnp.concatenate(parts, axis=0)
                else:
                    kg = k_ref[pl.ds(kb - 16, nk), cols]
                sts.append(jax.lax.dot_general(kg, qm, _NT, preferred_element_type=f32))
            mxs = {}

            def keep(j, pp, t, sm):
                c = (2 * j + pp) * 128
                st_ref[z, 16 * t:16 * t + 16, c:c + 128] = sm
                m8 = jnp.maximum(sm[0:8], sm[8:16])
                mxs[j, pp] = jnp.maximum(mxs[j, pp], m8) if (j, pp) in mxs else m8

            for t in range(ns // 16):
                for j in range(2):
                    hb = 2 * i + j
                    for pp in range(2):
                        pc = slice(pp * 128, pp * 128 + 128)
                        if not is_a:
                            c2 = row16 + 16 * t
                            dist = ql16 + 16 - c2
                            ok = (dist >= 0) & (dist < 16) & ((dist & 1) == 0)
                            if t == 0:
                                ok = ok & (hb >= 1)
                            sm = jnp.where(ok, sts[j][16 * t:16 * t + 16, pc], NEG)
                        elif t < HQ // 16:
                            s_old = jnp.where(hb >= 4, sts[j][32 * t:32 * t + 16, pc], NEG)
                            sm = jnp.where(row16 + 16 * t <= ql16,
                                           sts[j][32 * t + 16:32 * t + 32, pc], s_old)
                        else:
                            sm = jnp.where(hb >= 4 - 16 * t // HQ,
                                           sts[j][HQ + 16 * t:HQ + 16 * t + 16, pc], NEG)
                        keep(j, pp, t, sm)
            for (j, pp), m in mxs.items():
                c = (2 * j + pp) * 128
                mx_ref[z, :, c:c + 128] = jnp.broadcast_to(
                    jnp.max(m, axis=0, keepdims=True), (8, QB))

        def finish_rows(r):
            x = xr_ref[r, :]
            xn_ref[r, :] = x.astype(bf16) if last else layernorm(x)

        def body(i, c, first=False):
            if last and not first:
                pl.when(i >= 3)(lambda: out_cp(i - 3).start())
            if not first:
                finish_rows(pl.ds(pl.multiple_of(jnp.maximum(i - 2, 0) * QB, QB), QB))
            r0 = pl.multiple_of(i * QB, QB)
            rp = pl.ds(pl.multiple_of(jnp.maximum(i - 1, 0) * QB, QB), QB)
            v0 = pl.multiple_of(r0 + PAD - (WA if is_a else QB), QB)

            def sm_pv(g, slot, mid):
                st_ref, mx_ref = st_refs[g % 2], mx_refs[g % 2]
                z = i >> 12
                ots = []
                for pp in range(2):
                    if pp == 1:
                        mid()
                    pes, invs = [], []
                    for j in range(2):
                        c = (2 * j + pp) * 128
                        pe = jnp.exp2(st_ref[z, 0:ns, c:c + 128] - mx_ref[z, 0:1, c:c + 128])
                        invs.append(1.0 / jnp.sum(pe, axis=0, keepdims=True))
                        if is_a:
                            tri = row_q <= (lane_q2 & (HQ - 1))
                            pe = jnp.concatenate([jnp.where(tri, 0.0, pe[0:HQ]), pe[HQ:],
                                                  jnp.where(tri, pe[0:HQ], 0.0)], axis=0)
                        pes.append(pe)
                    for e in range(2):
                        h = g * 4 + 2 * pp + e
                        pieces = []
                        if nv > nk + HQ:
                            pieces.append(jnp.zeros((nv - nk - HQ, QB), f32))
                        m = (lane[0:1] >= HQ) if e else (lane[0:1] < HQ)
                        pieces += [jnp.where(m, pes[0][0:HQ], 0.0),
                                   jnp.where(m, pes[0][HQ:], pes[1][0:nk - HQ]),
                                   jnp.where(m, 0.0, pes[1][nk - HQ:])]
                        p = jnp.concatenate(pieces, axis=0).astype(bf16)
                        vth = vt_ref[h * DH:(h + 1) * DH, pl.ds(v0, nv)]
                        ot = jnp.dot(vth, p, preferred_element_type=f32)
                        ots.append(ot * jnp.where(m, invs[0], invs[1]))
                y = jnp.concatenate(ots, axis=0).T
                odd = (lane_q2 & DH) != 0
                y = jnp.concatenate([jnp.where(odd, y[HQ:], y[0:HQ]),
                                     jnp.where(odd, y[0:HQ], y[HQ:])], axis=0)
                o_ref[slot, :, g * 128:(g + 1) * 128] = y.astype(bf16)

            slot = i % 2
            for g in range(NG):
                if g + 1 < NG:
                    qk(i, g + 1)
                def outproj(g=g):
                    if first:
                        return
                    cols = slice(g * 128, (g + 1) * 128)
                    y = jnp.dot(o_ref[1 - slot], wo_ref[:, cols], preferred_element_type=f32)
                    xr_ref[rp, cols] = xr_ref[rp, cols] + y
                sm_pv(g, slot, outproj)
            qk(jnp.minimum(i + 1, S // QB - 1), 0)
            return c
        qk(pl.program_id(0), 0)
        body(pl.program_id(0), 0, first=True)
        jax.lax.fori_loop(1, S // QB, body, 0)
        if last:
            out_cp(S // QB - 3).start()
        finish_rows(pl.ds(S - 2 * QB, QB))
        if last:
            out_cp(S // QB - 2).start()
        r = pl.ds(S - QB, QB)
        xr_ref[r, :] = xr_ref[r, :] + jnp.dot(o_ref[(S // QB - 1) % 2], wo_ref[...],
                                              preferred_element_type=f32)
        finish_rows(r)
        if last:
            out_cp(S // QB - 1).start()
            pltpu.make_async_copy(xn_ref, out_hbm, out_sem).wait()

    w_cp[2].wait()
    qkv_phase(awqkv_ref, first=True)
    awo_cp.wait()
    attn_phase(awo_ref, True, False)
    bw_cp.wait()
    bwo_cp.wait()
    qkv_phase(bwqkv_ref)
    attn_phase(bwo_ref, False, False)
    qkv_phase(awqkv_ref)
    attn_phase(awo_ref, True, False)
    qkv_phase(bwqkv_ref)
    attn_phase(bwo_ref, False, True)


@jax.jit
def pallas_interleave_layers__sliding_block__sliding_local_dilated__prompt_kernel(
    A_x: jax.Array,
    A_wqkv: jax.Array,
    A_wo: jax.Array,
    B_x: jax.Array,
    B_wqkv: jax.Array,
    B_wo: jax.Array,
):
    del B_x
    x = A_x.reshape(S, D)
    out = pl.pallas_call(
        _kernel,
        grid=(1,),
        in_specs=[pl.BlockSpec(memory_space=pl.ANY)] * 5,
        out_specs=pl.BlockSpec(memory_space=pl.ANY),
        out_shape=jax.ShapeDtypeStruct((S, D), jnp.bfloat16),
        scratch_shapes=[
            pltpu.VMEM((D, 3 * D), jnp.bfloat16),
            pltpu.VMEM((D, D), jnp.bfloat16),
            pltpu.VMEM((D, 3 * D), jnp.bfloat16),
            pltpu.VMEM((D, D), jnp.bfloat16),
            pltpu.SemaphoreType.DMA((S // MB + 7,)),
            pltpu.VMEM((S, D), jnp.float32),
            pltpu.VMEM((S, D), jnp.bfloat16),
            pltpu.VMEM((S, D), jnp.bfloat16),
            pltpu.VMEM((PAD + S, D), jnp.bfloat16),
            pltpu.VMEM((D, PAD + S), jnp.bfloat16),
            pltpu.VMEM((2, 2 * QB, 4 * QB), jnp.float32),
            pltpu.VMEM((2, 2 * QB, 4 * QB), jnp.float32),
            pltpu.VMEM((2, 8, 4 * QB), jnp.float32),
            pltpu.VMEM((2, 8, 4 * QB), jnp.float32),
            pltpu.VMEM((2, QB, D), jnp.bfloat16),
        ],
        compiler_params=pltpu.CompilerParams(vmem_limit_bytes=100 * 1024 * 1024),
    )(x, A_wqkv, A_wo, B_wqkv, B_wo)
    return out.reshape(1, S, D)
```

```python
import math

import jax
import jax.numpy as jnp
import jax.experimental.pallas as pl
import jax.experimental.pallas.tpu as pltpu

S = 2048
D = 1024
H = 32
DH = 32
WA = 256
PAD = 256
QB = 128
HQ = 64
MB = 512
NEG = -1e9
LOG2E = 1.4426950408889634
QSCALE = (DH ** -0.5) * LOG2E

_NT = (((1,), (1,)), ((), ()))
_TN = (((0,), (0,)), ((), ()))


def _kernel(x_hbm, awqkv_hbm, awo_hbm, bwqkv_hbm, bwo_hbm, out_hbm,
            awqkv_ref, awo_ref, bwqkv_ref, bwo_ref, sems,
            xr_ref, xn_ref, q_ref, k_ref, vt_ref, st0_ref, st1_ref, mx0_ref, mx1_ref, o_ref, ob_ref):
    st_refs, mx_refs = (st0_ref, st1_ref), (mx0_ref, mx1_ref)
    f32, bf16 = jnp.float32, jnp.bfloat16

    nxc = S // MB
    x_cp = [pltpu.make_async_copy(x_hbm.at[c * MB:(c + 1) * MB], xn_ref.at[c * MB:(c + 1) * MB],
                                  sems.at[c]) for c in range(nxc)]
    w_cp = [pltpu.make_async_copy(awqkv_hbm.at[:, t * D:(t + 1) * D],
                                  awqkv_ref.at[:, t * D:(t + 1) * D], sems.at[nxc + t])
            for t in range(3)]
    awo_cp = pltpu.make_async_copy(awo_hbm, awo_ref, sems.at[nxc + 3])
    bw_cp = pltpu.make_async_copy(bwqkv_hbm, bwqkv_ref, sems.at[nxc + 4])
    bwo_cp = pltpu.make_async_copy(bwo_hbm, bwo_ref, sems.at[nxc + 5])
    out_sem = sems.at[nxc + 6]

    def out_cp(blk):
        r = pl.ds(pl.multiple_of(blk * QB, QB), QB)
        return pltpu.make_async_copy(xn_ref.at[r], out_hbm.at[r], out_sem)

    x_cp[0].start()
    w_cp[2].start()
    for c in range(1, nxc):
        x_cp[c].start()
    w_cp[0].start()
    w_cp[1].start()

    k_ref[0:PAD, :] = jnp.zeros((PAD, D), bf16)
    vt_ref[:, 0:PAD] = jnp.zeros((D, PAD), bf16)

    def layernorm(x):
        m = jnp.mean(x, axis=-1, keepdims=True)
        xc = x - m
        v = jnp.mean(xc * xc, axis=-1, keepdims=True)
        return (xc * jax.lax.rsqrt(v + 1e-5)).astype(bf16)

    def load_x(i, c):
        r = pl.ds(pl.multiple_of(i * QB, QB), QB)
        x = xn_ref[r, :].astype(f32)
        xr_ref[r, :] = x
        xn_ref[r, :] = layernorm(x)
        return c
    for c in range(nxc):
        x_cp[c].wait()
        jax.lax.fori_loop(c * (MB // QB), (c + 1) * (MB // QB), load_x, 0)
    awo_cp.start()
    bw_cp.start()
    bwo_cp.start()

    def qkv_phase(w_ref, first=False):
        def body(i, c):
            r0 = pl.multiple_of(i * MB, MB)
            xn = xn_ref[pl.ds(r0, MB), :]
            vv = jnp.dot(xn, w_ref[:, 2 * D:3 * D], preferred_element_type=f32)
            vt_ref[:, pl.ds(PAD + r0, MB)] = vv.astype(bf16).T
            if first:
                pl.when(i == 0)(lambda: (w_cp[0].wait(), w_cp[1].wait()) and None)
            q = jnp.dot(xn, w_ref[:, 0:D], preferred_element_type=f32)
            q_ref[pl.ds(r0, MB), :] = (q * QSCALE).astype(bf16)
            k = jnp.dot(xn, w_ref[:, D:2 * D], preferred_element_type=f32)
            k_ref[pl.ds(PAD + r0, MB), :] = k.astype(bf16)
            return c
        jax.lax.fori_loop(0, S // MB, body, 0)

    lane = jax.lax.broadcasted_iota(jnp.int32, (QB, QB), 1)
    row = jax.lax.broadcasted_iota(jnp.int32, (QB, QB), 0)

    NG = H // 4
    lane_q = jax.lax.broadcasted_iota(jnp.int32, (HQ // 2, QB), 1)
    lane_q2 = jax.lax.broadcasted_iota(jnp.int32, (HQ, QB), 1)
    row_q = jax.lax.broadcasted_iota(jnp.int32, (HQ, QB), 0)
    ql16 = jax.lax.broadcasted_iota(jnp.int32, (16, QB), 1) & (HQ - 1)
    row16 = jax.lax.broadcasted_iota(jnp.int32, (16, QB), 0)

    def attn_phase(wo_ref, is_a, last):
        nk = HQ + WA if is_a else HQ + 16
        ns = WA if is_a else nk
        nv = QB + WA if is_a else 2 * QB

        def qk(i, g):
            r0 = pl.multiple_of(i * QB, QB)
            st_ref, mx_ref = st_refs[g % 2], mx_refs[g % 2]
            z = i >> 11
            cols = slice(g * 128, (g + 1) * 128)
            sts = []
            for j in range(2):
                qu = pltpu.bitcast(q_ref[pl.ds(r0 + HQ * j, HQ), cols], jnp.uint32)
                qm = jnp.concatenate(
                    [pltpu.bitcast(jnp.where((lane_q >> 5) == (hh ^ j), qu, jnp.uint32(0)), bf16)
                     for hh in range(4)], axis=0)
                kb = r0 + PAD + HQ * j
                if is_a:
                    k_old = k_ref[pl.ds(kb - WA, HQ), cols]
                    k_dia = k_ref[pl.ds(kb, HQ), cols]
                    parts = []
                    for t in range(HQ // 16):
                        parts += [k_old[16 * t:16 * t + 16], k_dia[16 * t:16 * t + 16]]
                    parts.append(k_ref[pl.ds(kb - WA + HQ, WA - HQ), cols])
                    kg = jnp.concatenate(parts, axis=0)
                else:
                    kg = k_ref[pl.ds(kb - 16, nk), cols]
                sts.append(jax.lax.dot_general(kg, qm, _NT, preferred_element_type=f32))
            mxs = {}

            def keep(j, pp, t, sm):
                c = (2 * j + pp) * 128
                st_ref[z, 16 * t:16 * t + 16, c:c + 128] = sm
                m8 = jnp.maximum(sm[0:8], sm[8:16])
                mxs[j, pp] = jnp.maximum(mxs[j, pp], m8) if (j, pp) in mxs else m8

            for t in range(ns // 16):
                for j in range(2):
                    hb = 2 * i + j
                    for pp in range(2):
                        pc = slice(pp * 128, pp * 128 + 128)
                        if not is_a:
                            c2 = row16 + 16 * t
                            dist = ql16 + 16 - c2
                            ok = (dist >= 0) & (dist < 16) & ((dist & 1) == 0)
                            if t == 0:
                                ok = ok & (hb >= 1)
                            sm = jnp.where(ok, sts[j][16 * t:16 * t + 16, pc], NEG)
                        elif t < HQ // 16:
                            s_old = jnp.where(hb >= 4, sts[j][32 * t:32 * t + 16, pc], NEG)
                            sm = jnp.where(row16 + 16 * t <= ql16,
                                           sts[j][32 * t + 16:32 * t + 32, pc], s_old)
                        else:
                            sm = jnp.where(hb >= 4 - 16 * t // HQ,
                                           sts[j][HQ + 16 * t:HQ + 16 * t + 16, pc], NEG)
                        keep(j, pp, t, sm)
            for (j, pp), m in mxs.items():
                c = (2 * j + pp) * 128
                mx_ref[z, :, c:c + 128] = jnp.broadcast_to(
                    jnp.max(m, axis=0, keepdims=True), (8, QB))

        def finish_rows(r):
            x = xr_ref[r, :]
            xn_ref[r, :] = x.astype(bf16) if last else layernorm(x)

        def body(i, c, first=False):
            if last and not first:
                pl.when(i >= 3)(lambda: out_cp(i - 3).start())
            if not first:
                finish_rows(pl.ds(pl.multiple_of(jnp.maximum(i - 2, 0) * QB, QB), QB))
            r0 = pl.multiple_of(i * QB, QB)
            rp = pl.ds(pl.multiple_of(jnp.maximum(i - 1, 0) * QB, QB), QB)
            v0 = pl.multiple_of(r0 + PAD - (WA if is_a else QB), QB)

            def sm_pv(g, slot, mid):
                st_ref, mx_ref = st_refs[g % 2], mx_refs[g % 2]
                z = i >> 12
                ots = []
                for pp in range(2):
                    if pp == 1:
                        mid()
                    pes, invs = [], []
                    for j in range(2):
                        c = (2 * j + pp) * 128
                        pe = jnp.exp2(st_ref[z, 0:ns, c:c + 128] - mx_ref[z, 0:1, c:c + 128])
                        invs.append(1.0 / jnp.sum(pe, axis=0, keepdims=True))
                        if is_a:
                            tri = row_q <= (lane_q2 & (HQ - 1))
                            pe = jnp.concatenate([jnp.where(tri, 0.0, pe[0:HQ]), pe[HQ:],
                                                  jnp.where(tri, pe[0:HQ], 0.0)], axis=0)
                        pes.append(pe)
                    for e in range(2):
                        h = g * 4 + 2 * pp + e
                        pieces = []
                        if nv > nk + HQ:
                            pieces.append(jnp.zeros((nv - nk - HQ, QB), f32))
                        m = (lane[0:1] >= HQ) if e else (lane[0:1] < HQ)
                        pieces += [jnp.where(m, pes[0][0:HQ], 0.0),
                                   jnp.where(m, pes[0][HQ:], pes[1][0:nk - HQ]),
                                   jnp.where(m, 0.0, pes[1][nk - HQ:])]
                        p = jnp.concatenate(pieces, axis=0).astype(bf16)
                        vth = vt_ref[h * DH:(h + 1) * DH, pl.ds(v0, nv)]
                        ot = jnp.dot(vth, p, preferred_element_type=f32)
                        ots.append(ot * jnp.where(m, invs[0], invs[1]))
                y = jnp.concatenate(ots, axis=0).T
                odd = (lane_q2 & DH) != 0
                y = jnp.concatenate([jnp.where(odd, y[HQ:], y[0:HQ]),
                                     jnp.where(odd, y[0:HQ], y[HQ:])], axis=0)
                if is_a:
                    o_ref[slot, :, g * 128:(g + 1) * 128] = y.astype(bf16)
                else:
                    ob_ref[pl.ds(r0, QB), g * 128:(g + 1) * 128] = y.astype(bf16)

            slot = i % 2
            for g in range(NG):
                if g + 1 < NG:
                    qk(i, g + 1)
                def outproj(g=g):
                    if first:
                        return
                    cols = slice(g * 128, (g + 1) * 128)
                    y = jnp.dot(o_ref[1 - slot], wo_ref[:, cols], preferred_element_type=f32)
                    xr_ref[rp, cols] = xr_ref[rp, cols] + y
                sm_pv(g, slot, outproj)
            qk(jnp.minimum(i + 1, S // QB - 1), 0)
            return c
        qk(pl.program_id(0), 0)
        if is_a:
            body(pl.program_id(0), 0, first=True)
            jax.lax.fori_loop(1, S // QB, body, 0)
            finish_rows(pl.ds(S - 2 * QB, QB))
            r = pl.ds(S - QB, QB)
            xr_ref[r, :] = xr_ref[r, :] + jnp.dot(o_ref[(S // QB - 1) % 2], wo_ref[...],
                                                  preferred_element_type=f32)
            finish_rows(r)
            return
        jax.lax.fori_loop(0, S // QB, lambda i, c: body(i, c, first=True), 0)

        PB = 2 * QB

        def proj(i, c, first=False):
            if not first:
                if last:
                    pl.when(i >= 2)(lambda: (out_cp(2 * i - 4).start(),
                                             out_cp(2 * i - 3).start()) and None)
                finish_rows(pl.ds(pl.multiple_of((i - 1) * PB, PB), PB))
            r = pl.ds(pl.multiple_of(i * PB, PB), PB)
            xr_ref[r, :] = xr_ref[r, :] + jnp.dot(ob_ref[r, :], wo_ref[...],
                                                  preferred_element_type=f32)
            return c
        proj(0, 0, first=True)
        jax.lax.fori_loop(1, S // PB, proj, 0)
        if last:
            out_cp(S // QB - 4).start()
            out_cp(S // QB - 3).start()
        finish_rows(pl.ds(S - PB, PB))
        if last:
            out_cp(S // QB - 2).start()
            out_cp(S // QB - 1).start()
            pltpu.make_async_copy(xn_ref, out_hbm, out_sem).wait()

    w_cp[2].wait()
    qkv_phase(awqkv_ref, first=True)
    awo_cp.wait()
    attn_phase(awo_ref, True, False)
    bw_cp.wait()
    bwo_cp.wait()
    qkv_phase(bwqkv_ref)
    attn_phase(bwo_ref, False, False)
    qkv_phase(awqkv_ref)
    attn_phase(awo_ref, True, False)
    qkv_phase(bwqkv_ref)
    attn_phase(bwo_ref, False, True)


@jax.jit
def pallas_interleave_layers__sliding_block__sliding_local_dilated__prompt_kernel(
    A_x: jax.Array,
    A_wqkv: jax.Array,
    A_wo: jax.Array,
    B_x: jax.Array,
    B_wqkv: jax.Array,
    B_wo: jax.Array,
):
    del B_x
    x = A_x.reshape(S, D)
    out = pl.pallas_call(
        _kernel,
        grid=(1,),
        in_specs=[pl.BlockSpec(memory_space=pl.ANY)] * 5,
        out_specs=pl.BlockSpec(memory_space=pl.ANY),
        out_shape=jax.ShapeDtypeStruct((S, D), jnp.bfloat16),
        scratch_shapes=[
            pltpu.VMEM((D, 3 * D), jnp.bfloat16),
            pltpu.VMEM((D, D), jnp.bfloat16),
            pltpu.VMEM((D, 3 * D), jnp.bfloat16),
            pltpu.VMEM((D, D), jnp.bfloat16),
            pltpu.SemaphoreType.DMA((S // MB + 7,)),
            pltpu.VMEM((S, D), jnp.float32),
            pltpu.VMEM((S, D), jnp.bfloat16),
            pltpu.VMEM((S, D), jnp.bfloat16),
            pltpu.VMEM((PAD + S, D), jnp.bfloat16),
            pltpu.VMEM((D, PAD + S), jnp.bfloat16),
            pltpu.VMEM((2, 2 * QB, 4 * QB), jnp.float32),
            pltpu.VMEM((2, 2 * QB, 4 * QB), jnp.float32),
            pltpu.VMEM((2, 8, 4 * QB), jnp.float32),
            pltpu.VMEM((2, 8, 4 * QB), jnp.float32),
            pltpu.VMEM((2, QB, D), jnp.bfloat16),
            pltpu.VMEM((S, D), jnp.bfloat16),
        ],
        compiler_params=pltpu.CompilerParams(vmem_limit_bytes=100 * 1024 * 1024),
    )(x, A_wqkv, A_wo, B_wqkv, B_wo)
    return out.reshape(1, S, D)
```
